```python
import os as _os
_os.environ.setdefault("JAX_PLATFORMS", "cpu")
import jax
import jax.numpy as jnp

def _softmax(x, axis=-1):
    return jax.nn.softmax(x, axis=axis)
def _gelu(x):
    return jax.nn.gelu(x, approximate=True)
def _silu(x):
    return jax.nn.silu(x)
def _sigmoid(x):
    return jax.nn.sigmoid(x)
def _layernorm(x, axis=-1, eps=1e-5):
    m = jnp.mean(x, axis=axis, keepdims=True)
    v = jnp.var(x, axis=axis, keepdims=True)
    return (x - m) / jnp.sqrt(v + eps)
def _scatter_add(tgt, idx, src, axis=0):
    return tgt.at[idx].add(src)
def _segment_sum(src, seg, n):
    return jax.ops.segment_sum(src, seg, n)
class _Rng:
    def __init__(self, key):
        self._k = key
    def _next(self):
        self._k, sub = jax.random.split(self._k)
        return sub
    def normal(self, shape):
        return jax.random.normal(self._next(), shape, dtype=jnp.bfloat16)
    def randint(self, lo, hi, shape):
        return jax.random.randint(self._next(), shape, lo, hi, dtype=jnp.int32)
    def uniform(self, shape, lo=0.0, hi=1.0):
        return jax.random.uniform(self._next(), shape, jnp.bfloat16, lo, hi)
    def permutation(self, n):
        return jax.random.permutation(self._next(), n)


kernel_name = 'standalone__sliding_block_cached__sampling'

def setup_inputs():
    _rng = _Rng(jax.random.key(int.from_bytes(__import__("os").urandom(4), "little")))
    _w = (lambda a: (lambda t: t.astype(jnp.bfloat16) if jnp.issubdtype(t.dtype, jnp.floating) else t)(jnp.asarray(a)))
    B, Sq, D = 8, 16, 576
    Hq, Hkv, Sk, Dh = 32, 16, 8192, 128
    assert Hq % Hkv == 0, (Hq, Hkv)
    return {
        "x": _w((lambda *s: _rng.normal(s) * 0.8)(B, Sq, D)),
        "k_cache": _w((lambda *s: _rng.normal(s) * 0.8)(B, Hkv, Sk, Dh)),
        "v_cache": _w((lambda *s: _rng.normal(s) * 0.05)(B, Hkv, Sk, Dh)),
        "wq": _w((lambda *s: _rng.normal(s) * 0.8)(D, Hq * Dh) * (D ** -0.5)),
        "wo": _w((lambda *s: _rng.normal(s) * 0.05)(Hq * Dh, D) * ((Hq * Dh) ** -0.5)),
    }

def reference(x, k_cache, v_cache, wq, wo):
    B, Sq, D = x.shape
    Hq, Dh = 32, 128
    Hkv, Sk = k_cache.shape[1], k_cache.shape[2]
    W = min(4096, max(256, Sk // 4))
    rep = Hq // Hkv
    q = (lambda x, *d: x.transpose(*d))((x @ wq).reshape(B, Sq, Hq, Dh), 0, 2, 1, 3)
    k = jnp.repeat(k_cache[:, :, Sk - W:, :], rep, axis=1)
    v = jnp.repeat(v_cache[:, :, Sk - W:, :], rep, axis=1)
    scores = jnp.einsum("bhqd,bhkd->bhqk", q, k) * (Dh ** -0.5)
    p = _softmax(scores, axis=-1)
    o = jnp.einsum("bhqk,bhkd->bhqd", p, v)
    return (lambda x, *d: x.transpose(*d))(o, 0, 2, 1, 3).reshape(B, Sq, Hq * Dh) @ wo
```

```python
import math

import jax
import jax.numpy as jnp
from jax import lax
import jax.experimental.pallas as pl
import jax.experimental.pallas.tpu as pltpu

_HQ = 32
_DH = 128
_TILE = 128
_RUN = 32
_SLOTS = 4
_WBLK = 512

_SMALL_K = (3, 4)
_SMALL_V = (2, 7)
_SMALL_WQ = (4, 4)
_SMALL_WO = 4
_GAP_NS = 50

_NT = (((1,), (1,)), ((), ()))
_F32 = jnp.float32


def _ds(start, size):
    if not isinstance(start, int):
        start = pl.multiple_of(start, size)
    return pl.ds(start, size)


def _kernel(
    x_hbm, k_hbm, v_hbm, wq_hbm, wot_hbm, o_hbm,
    x_s, wq_s, wot_s, q_s, k_s, v_s, p_s, m_s, l_s, alpha_s, acc_s, att_s, out_s,
    x_sem, wq_sem, kv_sem, wo_sem, out_sem,
    *, window,
):
    batch, half_heads, _, sk, dh = k_hbm.shape
    hkv = 2 * half_heads
    rows, d = x_hbm.shape
    sq = rows // batch
    dtype = x_s.dtype
    tiles = window // _TILE
    steps = batch * tiles
    n_wq = wq_hbm.shape[1] // _WBLK
    exp2_scale = dh ** -0.5 * math.log2(math.e)

    order = [
        (e, 2 * _RUN * i + _RUN * j)
        for i in range(_TILE // (2 * _RUN)) for e in range(2) for j in range(2)
    ]
    n_small = (sum(_SMALL_K), sum(_SMALL_V))

    def unit(i):
        if isinstance(i, int):
            return i // tiles, sk - window + (i % tiles) * _TILE, i % _SLOTS
        b = lax.shift_right_logical(i, tiles.bit_length() - 1)
        return b, sk - window + (i & (tiles - 1)) * _TILE, i & (_SLOTS - 1)

    def kv_bulk(i, a):
        b, r0, slot = unit(i)
        for n, (e, off) in enumerate(order):
            cut = len(range(n, n_small[a], len(order)))
            heads = pl.ds(cut, half_heads - cut)
            pltpu.make_async_copy(
                (k_hbm, v_hbm)[a].at[b, heads, e, _ds(r0 + off, _RUN), :],
                (k_s, v_s)[a].at[slot, heads, e, pl.ds(off, _RUN), :],
                kv_sem.at[a, slot],
            ).start(priority=1)

    def kv_small(i, a, t):
        b, r0, slot = unit(i)
        e, off = order[t % len(order)]
        h = t // len(order)
        pltpu.make_async_copy(
            (k_hbm, v_hbm)[a].at[b, h, e, _ds(r0 + off, _RUN), :],
            (k_s, v_s)[a].at[slot, h, e, pl.ds(off, _RUN), :],
            kv_sem.at[a, slot],
        ).start(priority=0)

    def kv_wait(i, a):
        slot = unit(i)[2]
        buf = (k_s, v_s)[a].at[slot]
        pltpu.make_async_copy(buf, buf, kv_sem.at[a, slot]).wait()

    def wq_copy(u, r):
        return pltpu.make_async_copy(
            wq_hbm.at[r, _ds(u * _WBLK, _WBLK)], wq_s.at[u, r, :], wq_sem.at[u]
        )

    def wq_bulk(u):
        skip = 8 * sum(_SMALL_WQ)
        wq_copy(u, pl.ds(skip, d - skip)).start(priority=1)

    def wq_small(u, t):
        wq_copy(u, pl.ds(8 * t, 8)).start(priority=0)

    def wq_wait(u):
        pltpu.make_async_copy(wq_s.at[u], wq_s.at[u], wq_sem.at[u]).wait()

    hd = wot_hbm.shape[1]
    chunks = [(r, min(128, d - r)) for r in range(0, d, 128)]
    chunks = chunks[-1:] + chunks[:-1]
    splits = [1] * (len(chunks) - 2) + [2, 4]
    pieces = [
        (r, nr, c, hd // n)
        for (r, nr), n in zip(chunks, splits) for c in range(0, hd, hd // n)
    ]

    def wo_rects(u):
        r, nr, c, nc = pieces[u]
        n = max(1, round(_SMALL_WO * nr * nc / (64 * hd)))
        per = nc // _WBLK
        strips = -(-n // per)
        small = [
            (r + 8 * (t // per), 8, c + _WBLK * (t % per), _WBLK) for t in range(n)
        ]
        bulk = [(r + 8 * strips, nr - 8 * strips, c, nc)]
        if n % per:
            used = _WBLK * (n % per)
            bulk.append((r + 8 * (strips - 1), 8, c + used, nc - used))
        return bulk, small

    def wo_copy(u, rect):
        r, c = pl.ds(rect[0], rect[1]), pl.ds(rect[2], rect[3])
        return pltpu.make_async_copy(wot_hbm.at[r, c], wot_s.at[r, c], wo_sem.at[u])

    def wo_bulk(lo, hi):
        for u in range(lo, hi):
            for rect in wo_rects(u)[0]:
                wo_copy(u, rect).start(priority=1)

    wo_smalls = [(u, rect) for u in range(len(pieces)) for rect in wo_rects(u)[1]]

    def wo_small(t):
        if t < len(wo_smalls):
            wo_copy(*wo_smalls[t]).start(priority=0)

    def out_copy(r, nr):
        c = pl.ds(r, nr)
        return pltpu.make_async_copy(
            out_s.at[:, c], o_hbm.at[:, c], out_sem.at[r // 128]
        )

    def reset_state():
        m_s[...] = jnp.full(m_s.shape, -jnp.inf, _F32)
        l_s[...] = jnp.zeros(l_s.shape, _F32)
        acc_s[...] = jnp.zeros(acc_s.shape, _F32)

    def with_small_dmas(counts, small, matmul, update):
        during, after = counts
        at = [int((t + 0.5) * hkv / during) for t in range(during)]
        results = []
        for j in range(hkv):
            results.append(matmul(j))
            if j in at:
                small(at.index(j))
        for j in range(hkv):
            update(j, results[j])
        for t in range(during, during + after):
            pl.delay(_GAP_NS)
            small(t)

    def scores_step(i, small):
        b, _, slot = unit(i)

        def matmul(j):
            k = k_s[slot, j // 2, j % 2]
            return lax.dot_general(q_s[j, b], k, _NT, preferred_element_type=_F32)

        def update(j, s):
            m_old = m_s[j]
            m_new = jnp.maximum(m_old, jnp.max(s, axis=1, keepdims=True))
            alpha = jnp.exp2((m_old - m_new) * exp2_scale)
            p = jnp.exp2((s - m_new) * exp2_scale)
            m_s[j] = m_new
            alpha_s[j] = alpha
            l_s[j] = alpha * l_s[j] + p
            p_s[j] = p.astype(dtype)

        with_small_dmas(_SMALL_K, small, matmul, update)

    def values_step(i, small):
        slot = unit(i)[2]

        def matmul(j):
            v = v_s[slot, j // 2, j % 2]
            return jnp.dot(p_s[j], v, preferred_element_type=_F32)

        def update(j, pv):
            acc_s[j] = alpha_s[j] * acc_s[j] + pv

        with_small_dmas(_SMALL_V, small, matmul, update)

    def finish_batch(b):
        per = _WBLK // dh
        for j in range(hkv):
            o = acc_s[j] / jnp.sum(l_s[j], axis=1, keepdims=True)
            o = o.astype(dtype)
            for r in range(2):
                h = 2 * j + r
                att_s[h // per, b, :, pl.ds((h % per) * dh, dh)] = o[r * sq:(r + 1) * sq]
        reset_state()

    x_copy = pltpu.make_async_copy(x_hbm, x_s, x_sem)
    wq_bulk(0)
    x_copy.start()
    pl.delay(1)
    for u in range(1, n_wq):
        wq_bulk(u)
    pl.delay(1)
    kv_bulk(0, 0)
    pl.delay(1)
    kv_bulk(0, 1)
    for u in range(2):
        for t in range(sum(_SMALL_WQ)):
            pl.delay(_GAP_NS)
            wq_small(u, t)
    reset_state()
    x_copy.wait()

    def q_block(u, _):
        def small(t):
            pl.when(u < n_wq - 2)(lambda: wq_small(u + 2, t))
            for a in range(2):
                if t < n_small[a]:
                    pl.when(u == n_wq - 2 + a)(lambda: kv_small(0, a, t))

        wq_wait(u)
        pl.when(u == n_wq - 1)(lambda: kv_bulk(1, 0))
        for t in range(_SMALL_WQ[0]):
            small(t)
        q = jnp.dot(x_s[...], wq_s[u], preferred_element_type=_F32).astype(dtype)
        for c in range(_WBLK // dh):
            j = (_WBLK // (2 * dh)) * u + c // 2
            q_s[j, :, pl.ds((c % 2) * sq, sq), :] = (
                q[:, c * dh:(c + 1) * dh].reshape(batch, sq, dh)
            )
        for t in range(_SMALL_WQ[0], sum(_SMALL_WQ)):
            pl.delay(_GAP_NS)
            small(t)

    lax.fori_loop(0, n_wq, q_block, None)
    for a in range(2):
        for t in range(sum(_SMALL_WQ), n_small[a]):
            kv_small(0, a, t)

    def step(i, near_end):
        def small(a, t):
            if near_end:
                pl.when(i + 1 < steps)(lambda: kv_small(i + 1, a, t))
                pl.when(i + 1 == steps)(lambda: wo_small(a * n_small[0] + t))
            else:
                kv_small(i + 1, a, t)

        kv_wait(i, 0)
        if near_end:
            pl.when(i + 1 < steps)(lambda: kv_bulk(i + 1, 1))
            pl.when(i + 1 == steps)(lambda: wo_bulk(4, len(pieces)))
        else:
            kv_bulk(i + 1, 1)
        scores_step(i, lambda t: small(0, t))

        kv_wait(i, 1)
        if near_end:
            pl.when(i + 2 == steps)(lambda: wo_bulk(0, 4))
        else:
            kv_bulk(i + 2, 0)
        values_step(i, lambda t: small(1, t))

        pl.when((i & (tiles - 1)) == tiles - 1)(lambda: finish_batch(unit(i)[0]))

    lax.fori_loop(0, steps - 2, lambda i, _: step(i, False), None)
    lax.fori_loop(steps - 2, steps, lambda i, _: step(i, True), None)

    started = sum(n_small)
    waited = 0
    acc = None
    for u, (r, nr, c, nc) in enumerate(pieces):
        waited += len(wo_rects(u)[1])
        assert started >= waited
        todo = 0
        if u + 1 < len(pieces):
            ahead = waited + len(wo_rects(u + 1)[1]) + _SMALL_WO
            todo = max(0, min(len(wo_smalls), ahead) - started)
        during = min(todo, nc // 1024)
        wo_copy(u, pieces[u]).wait()
        for t in range(during):
            wo_small(started + t)
        att = jnp.concatenate(
            [
                att_s[n].reshape(rows, _WBLK)
                for n in range(c // _WBLK, (c + nc) // _WBLK)
            ],
            axis=1,
        )
        w = wot_s[pl.ds(r, nr), pl.ds(c, nc)]
        part = lax.dot_general(att, w, _NT, preferred_element_type=_F32)
        acc = part if c == 0 else acc + part
        if c + nc == hd:
            out_s[:, pl.ds(r, nr)] = acc.astype(out_s.dtype)
            out_copy(r, nr).start()
        for t in range(during, todo):
            pl.delay(_GAP_NS)
            wo_small(started + t)
        started += todo

    for r, nr in chunks:
        out_copy(r, nr).wait()


@jax.jit
def pallas_standalone__sliding_block_cached__sampling_kernel(
    x: jax.Array,
    k_cache: jax.Array,
    v_cache: jax.Array,
    wq: jax.Array,
    wo: jax.Array,
):
    batch, sq, d = x.shape
    _, hkv, sk, dh = k_cache.shape
    window = min(4096, max(256, sk // 4))
    assert dh == _DH and _HQ == 2 * hkv and window % _TILE == 0
    tiles = window // _TILE
    assert tiles & (tiles - 1) == 0
    rows, hd, dtype = batch * sq, _HQ * dh, x.dtype
    n_chunks = pl.cdiv(d, 128)

    def kernel(*refs):
        _kernel(*refs, window=window)

    hbm = pl.BlockSpec(memory_space=pl.ANY)
    kv_shape = (batch, hkv // 2, 2, sk, dh)
    state = pltpu.VMEM((hkv, 2 * sq, dh), _F32)
    out = pl.pallas_call(
        kernel,
        out_shape=jax.ShapeDtypeStruct((rows, d), dtype),
        in_specs=[hbm] * 5,
        out_specs=hbm,
        scratch_shapes=[
            pltpu.VMEM((rows, d), dtype),
            pltpu.VMEM((hd // _WBLK, d, _WBLK), dtype),
            pltpu.VMEM((d, hd), dtype),
            pltpu.VMEM((hkv, batch, 2 * sq, dh), dtype),
            pltpu.VMEM((_SLOTS, hkv // 2, 2, _TILE, dh), dtype),
            pltpu.VMEM((_SLOTS, hkv // 2, 2, _TILE, dh), dtype),
            pltpu.VMEM((hkv, 2 * sq, dh), dtype),
            state,
            state,
            state,
            state,
            pltpu.VMEM((hd // _WBLK, batch, sq, _WBLK), dtype),
            pltpu.VMEM((rows, d), dtype),
            pltpu.SemaphoreType.DMA,
            pltpu.SemaphoreType.DMA((hd // _WBLK,)),
            pltpu.SemaphoreType.DMA((2, _SLOTS)),
            pltpu.SemaphoreType.DMA((n_chunks + 4,)),
            pltpu.SemaphoreType.DMA((n_chunks,)),
        ],
        compiler_params=pltpu.CompilerParams(
            vmem_limit_bytes=48 * 1024 * 1024,
            disable_bounds_checks=True,
            disable_semaphore_checks=True,
        ),
        name="sliding_block_cached_sampling",
    )(
        x.reshape(rows, d),
        k_cache.reshape(kv_shape),
        v_cache.reshape(kv_shape),
        wq,
        wo.T,
    )
    return out.reshape(batch, sq, d)
```

```python
import functools
import math

import jax
import jax.numpy as jnp
from jax import lax
import jax.experimental.pallas as pl
import jax.experimental.pallas.tpu as pltpu

_HQ = 32
_TILE = 128
_RUN = 64
_HEADS_PER_DMA = 4
_SLOTS = 4
_WROWS = 64
_WCOLS = 512
_QUEUE = 26

_SMALL_KV = (5, 7)
_WQ_AHEAD = 24
_WQ_LEAD = 8
_WO_SPLITS = ((9, 7), (6, 5, 5))

_NT = (((1,), (1,)), ((), ()))
_F32 = jnp.float32


def _ds(start, size):
    if not isinstance(start, int):
        start = pl.multiple_of(start, size)
    return pl.ds(start, size)


def _wait(filled, sem):
    pltpu.make_async_copy(filled, filled, sem).wait()


def _plan_wo(d, hd, early_small):
    blocks = d // _WROWS
    chunks = [(b, min(2, blocks - b)) for b in range(0, blocks, 2)][::-1]
    splits = [(16,)] * (len(chunks) - len(_WO_SPLITS)) + list(_WO_SPLITS)
    pieces = []
    for (b0, nb), split in zip(chunks, splits):
        c = 0
        for part in split:
            nc = hd * part // 16
            pieces.append((b0, nb, c, nc, nc // _WCOLS if nc == hd else 0))
            c += nc

    firsts = [u for u, n in enumerate(early_small) for _ in range(n)]
    firsts += [u + 2 for u, piece in enumerate(pieces) for _ in range(piece[4])]
    taken = [0] * len(pieces)
    small = []
    for first in firsts:
        for u in range(first, len(pieces)):
            b0, nb, c, nc, _ = pieces[u]
            per_row = nc // _WCOLS
            if nc == hd and taken[u] < nb * per_row:
                r, k = divmod(taken[u], per_row)
                small.append((u, b0, 1, 8 * r, c + k * _WCOLS, _WCOLS))
                taken[u] += 1
                break
        else:
            small.append(None)

    bulk = []
    for u, (b0, nb, c, nc, _) in enumerate(pieces):
        full, part = divmod(taken[u], nc // _WCOLS)
        used = part * _WCOLS
        if nb == 1 or nc < hd // 2:
            for b in range(nb):
                r = 8 * full if b == 0 else 0
                if b == 0 and part:
                    bulk.append((u, b0, 1, r, 8, c + used, nc - used))
                    r += 8
                bulk.append((u, b0 + b, 1, r, _WROWS - r, c, nc))
            continue
        run = hd // 2 if nc % (hd // 2) == 0 else nc
        for r in range(0, _WROWS, 8):
            if r // 8 == full and part:
                bulk.append((u, b0, 1, r, 8, c + used, nc - used))
            if r // 8 < full + bool(part):
                bulk.append((u, b0 + 1, nb - 1, r, 8, c, nc))
            else:
                bulk += [(u, b0, nb, r, 8, k, run) for k in range(c, c + nc, run)]
    return pieces, bulk, small


def _kernel(
    x_hbm, k_hbm, v_hbm, wq_hbm, wot_hbm, o_hbm,
    x_s, wq_s, wot_s, kv_s, q_s, p_s, m_s, l_s, alpha_s, acc_s, att_s, part_s, out_s,
    x_sem, wq_sem, kv_sem, wo_sem, out_sem,
    *, window,
):
    batch, hkv, sk, dh = k_hbm.shape
    rows, d = x_hbm.shape
    hd = wq_hbm.shape[2]
    sq = rows // batch
    dtype = x_s.dtype
    tiles = window // _TILE
    steps = batch * tiles
    exp2_scale = dh ** -0.5 * math.log2(math.e)

    n_dmas = 2 * hkv // _HEADS_PER_DMA
    n_small = sum(_SMALL_KV)

    def locate(i):
        if isinstance(i, int):
            return i // tiles, i % tiles, i % _SLOTS
        b = lax.shift_right_logical(i, tiles.bit_length() - 1)
        return b, i & (tiles - 1), i & (_SLOTS - 1)

    def kv_copy(i, half, n, h0, nh, r0, nr):
        b, tile, slot = locate(i)
        group, a = divmod(n, 2)
        heads = pl.ds(group * _HEADS_PER_DMA + h0, nh)
        r = half * _RUN + r0
        src = (k_hbm, v_hbm)[a].at[
            b, heads, _ds(sk - window + tile * _TILE + r, nr), :
        ]
        dst = kv_s.at[slot, a, heads, pl.ds(r, nr), :]
        return pltpu.make_async_copy(src, dst, kv_sem.at[slot, half, n])

    def kv_bulk(i, half):
        for n in range(n_dmas):
            cut = len(range(n, n_small // 2, n_dmas))
            kv_copy(i, half, n, cut, _HEADS_PER_DMA - cut, 0, _RUN).start(priority=1)

    def kv_small(i, half, t):
        run, part = divmod(t, 2)
        kv_copy(
            i, half, run % n_dmas, run // n_dmas, 1, part * (_RUN // 2), _RUN // 2
        ).start(priority=0)

    def kv_wait(i, half, small=None):
        slot = locate(i)[2]
        first = n_dmas - 1 - _SMALL_KV[1]
        for n in range(n_dmas):
            group, a = divmod(n, 2)
            heads = pl.ds(group * _HEADS_PER_DMA, _HEADS_PER_DMA)
            _wait(
                kv_s.at[slot, a, heads, pl.ds(half * _RUN, _RUN), :],
                kv_sem.at[slot, half, n],
            )
            if small is not None and first <= n < n_dmas - 1:
                small(_SMALL_KV[0] + n - first)

    wq_dmas = [(r, c) for r in range(0, _WROWS, 8) for c in range(0, hd, _WCOLS)]
    w_blocks = d // _WROWS

    def wq_index(n, b0, nb):
        r, c = wq_dmas[n]
        return pl.ds(b0, nb), pl.ds(r, 8), pl.ds(c, _WCOLS)

    def wq_start(n, b0, nb, priority):
        ix = wq_index(n, b0, nb)
        pltpu.make_async_copy(wq_hbm.at[ix], wq_s.at[ix], wq_sem.at[n]).start(
            priority=priority
        )

    pieces, wo_bulk, wo_small = _plan_wo(d, hd, (n_small, n_small // 2))
    wo_bulk_total = len(wo_bulk)

    def wo_start(u, b0, nb, r, nr, c, nc, priority):
        ix = pl.ds(b0, nb), pl.ds(r, nr), pl.ds(c, nc)
        pltpu.make_async_copy(wot_hbm.at[ix], wot_s.at[ix], wo_sem.at[u]).start(
            priority=priority
        )

    def next_wo_bulk(count):
        for _ in range(min(count, len(wo_bulk))):
            wo_start(*wo_bulk.pop(0), priority=1)

    def next_wo_small(_=None):
        entry = wo_small.pop(0)
        if entry is not None:
            u, b0, nb, r, c, nc = entry
            wo_start(u, b0, nb, r, 8, c, nc, priority=0)

    def project_q(b, j0, nj):
        w = wq_s[:, :, _ds(j0 * 2 * dh, nj * 2 * dh)].reshape(d, nj * 2 * dh)
        q = jnp.dot(x_s[_ds(b * sq, sq), :], w, preferred_element_type=_F32)
        q = q.astype(dtype)
        for h in range(2 * nj):
            q_s[b & 1, j0 + h // 2, pl.ds((h % 2) * sq, sq), :] = (
                q[:, h * dh:(h + 1) * dh]
            )

    def reset_state():
        m_s[...] = jnp.full(m_s.shape, -jnp.inf, _F32)
        l_s[...] = jnp.zeros(l_s.shape, _F32)
        acc_s[...] = jnp.zeros(acc_s.shape, _F32)

    def all_matmuls(matmul, small, count):
        after = [int((t + 0.5) * hkv / count) for t in range(count)]
        results = []
        for j in range(hkv):
            results.append(matmul(j))
            if j in after:
                small(after.index(j))
        return results

    def scores_step(i, small, count=_SMALL_KV[0]):
        b, _, slot = locate(i)
        scores = all_matmuls(
            lambda j: lax.dot_general(
                q_s[b & 1, j], kv_s[slot, 0, j], _NT, preferred_element_type=_F32
            ),
            small,
            count,
        )
        for j, s in enumerate(scores):
            m_old = m_s[j]
            m_new = jnp.maximum(m_old, jnp.max(s, axis=1, keepdims=True))
            alpha = jnp.exp2((m_old - m_new) * exp2_scale)
            p = jnp.exp2((s - m_new) * exp2_scale)
            m_s[j] = m_new
            alpha_s[j] = alpha
            l_s[j] = alpha * l_s[j] + p
            p_s[j] = p.astype(dtype)

    def values_step(i, small, count=_SMALL_KV[0], next_q=True):
        b, tile, slot = locate(i)
        products = all_matmuls(
            lambda j: jnp.dot(
                p_s[j], kv_s[slot, 1, j], preferred_element_type=_F32
            ),
            small,
            count,
        )
        if next_q:
            project_q((b + 1) & (batch - 1), tile * (hkv // tiles), hkv // tiles)
        for j, pv in enumerate(products):
            acc_s[j] = alpha_s[j] * acc_s[j] + pv

    def finish_batch(b):
        for j in range(hkv):
            o = acc_s[j] / jnp.sum(l_s[j], axis=1, keepdims=True)
            o = o.astype(dtype)
            for h in range(2):
                att_s[j, b, :, pl.ds(h * dh, dh)] = o[h * sq:(h + 1) * sq]

    def wq_bulk(n):
        cut = int(n >= _WQ_LEAD)
        wq_start(n, cut, w_blocks - cut, priority=1)

    x_copy = pltpu.make_async_copy(x_hbm, x_s, x_sem)
    x_copy.start()
    for n in range(_WQ_AHEAD):
        wq_bulk(n)
    reset_state()
    units = [(0, 0), (0, 1), (1, 0)]
    small = [(i, half, t) for i, half in units for t in range(n_small)]
    small = small[:len(small) - _SMALL_KV[1]]
    for n in range(len(wq_dmas)):
        _wait(wq_s.at[wq_index(n, 0, w_blocks)], wq_sem.at[n])
        left = len(wq_dmas) - 1 - n
        if left >= _WQ_AHEAD:
            wq_bulk(n + _WQ_AHEAD)
        elif units and left + n_dmas * (4 - len(units)) <= _QUEUE:
            kv_bulk(*units.pop(0))
        if left >= _WQ_LEAD:
            wq_start(n + _WQ_LEAD, 0, 1, priority=0)
        else:
            kv_small(*small.pop(0))
    assert not units
    x_copy.wait()
    groups = 4
    for n in range(groups):
        for _ in range(-(-len(small) // (groups - n))):
            kv_small(*small.pop(0))
        project_q(0, n * hkv // groups, hkv // groups)
        if n == groups // 2 - 1:
            kv_wait(0, 0)
            kv_bulk(1, 1)
    assert not small

    def step(i, _):
        kv_wait(i, 1, functools.partial(kv_small, i + 1, 0))
        kv_bulk(i + 2, 0)
        scores_step(i, functools.partial(kv_small, i + 1, 1))
        kv_wait(i + 1, 0, functools.partial(kv_small, i + 1, 1))
        kv_bulk(i + 2, 1)
        values_step(i, functools.partial(kv_small, i + 2, 0))
        b, tile, _ = locate(i)

        @pl.when(tile == tiles - 1)
        def _():
            finish_batch(b)
            reset_state()

    lax.fori_loop(0, steps - 2, step, None)

    i = steps - 2
    kv_wait(i, 1, functools.partial(kv_small, i + 1, 0))
    next_wo_bulk(_QUEUE - 2 * n_dmas)
    scores_step(i, functools.partial(kv_small, i + 1, 1))
    kv_wait(i + 1, 0, functools.partial(kv_small, i + 1, 1))
    next_wo_bulk(n_dmas)
    values_step(i, next_wo_small, next_q=False)
    i = steps - 1
    kv_wait(i, 1, next_wo_small)
    next_wo_bulk(n_dmas)
    scores_step(i, next_wo_small, n_small // 4)
    values_step(i, next_wo_small, n_small // 4, next_q=False)
    finish_batch(batch - 1)

    def out_copy(n, c, nc):
        cols = pl.ds(c, nc)
        return pltpu.make_async_copy(
            out_s.at[:, cols], o_hbm.at[:, cols], out_sem.at[n]
        )

    def project_out(b0, nb, c, nc, m, nm):
        att = jnp.concatenate(
            [
                att_s[j, pl.ds(m // sq, nm // sq)].reshape(nm, 2 * dh)
                for j in range(c // (2 * dh), (c + nc) // (2 * dh))
            ],
            axis=1,
        )
        w = wot_s[pl.ds(b0, nb), :, pl.ds(c, nc)].reshape(nb * _WROWS, nc)
        return lax.dot_general(att, w, _NT, preferred_element_type=_F32)

    last = pieces[-1][1] * _WROWS
    all_bulk = _plan_wo(d, hd, (n_small, n_small // 2))[1]
    for u, (b0, nb, c, nc, count) in enumerate(pieces):
        assert all(entry[0] > u for entry in wo_bulk + wo_small if entry)
        _wait(wot_s.at[pl.ds(b0, nb), :, pl.ds(c, nc)], wo_sem.at[u])
        if u == len(pieces) - 1:
            out_copy(0, last, d - last).start()
        done = sum(entry[0] <= u for entry in all_bulk)
        next_wo_bulk(_QUEUE - (wo_bulk_total - len(wo_bulk) - done))
        total = None
        for k in range(nc // _WCOLS):
            if k < count:
                next_wo_small()
            part = project_out(b0, nb, c + k * _WCOLS, _WCOLS, 0, rows)
            total = part if total is None else total + part
        rest = nc % _WCOLS
        if rest:
            total += jnp.concatenate(
                [
                    project_out(b0, nb, c + nc - rest, rest, m, rows // 2)
                    for m in (0, rows // 2)
                ],
                axis=0,
            )
        if c > 0:
            total += part_s[...]
        if c + nc < hd:
            part_s[...] = total
        else:
            out_s[:, pl.ds(b0 * _WROWS, nb * _WROWS)] = total.astype(out_s.dtype)
    assert not wo_bulk and not wo_small
    out_copy(1, 0, last).start()
    out_copy(0, last, d - last).wait()
    out_copy(1, 0, last).wait()


@jax.jit
def pallas_standalone__sliding_block_cached__sampling_kernel(
    x: jax.Array,
    k_cache: jax.Array,
    v_cache: jax.Array,
    wq: jax.Array,
    wo: jax.Array,
):
    batch, sq, d = x.shape
    _, hkv, sk, dh = k_cache.shape
    window = min(4096, max(256, sk // 4))
    tiles = window // _TILE
    assert _HQ == 2 * hkv and d % _WROWS == 0 and window % _TILE == 0
    assert hkv % tiles == 0 and batch & (batch - 1) == 0
    rows, hd, dtype = batch * sq, _HQ * dh, x.dtype
    w_shape = (d // _WROWS, _WROWS, hd)

    hbm = pl.BlockSpec(memory_space=pl.ANY)
    state = pltpu.VMEM((hkv, 2 * sq, dh), _F32)
    out = pl.pallas_call(
        functools.partial(_kernel, window=window),
        out_shape=jax.ShapeDtypeStruct((rows, d), dtype),
        in_specs=[hbm] * 5,
        out_specs=hbm,
        scratch_shapes=[
            pltpu.VMEM((rows, d), dtype),
            pltpu.VMEM(w_shape, dtype),
            pltpu.VMEM(w_shape, dtype),
            pltpu.VMEM((_SLOTS, 2, hkv, _TILE, dh), dtype),
            pltpu.VMEM((2, hkv, 2 * sq, dh), dtype),
            pltpu.VMEM((hkv, 2 * sq, dh), dtype),
            state,
            state,
            state,
            state,
            pltpu.VMEM((hkv, batch, sq, 2 * dh), dtype),
            pltpu.VMEM((rows, 2 * _WROWS), _F32),
            pltpu.VMEM((rows, d), dtype),
            pltpu.SemaphoreType.DMA,
            pltpu.SemaphoreType.DMA((_WROWS // 8 * (hd // _WCOLS),)),
            pltpu.SemaphoreType.DMA((_SLOTS, 2, 2 * hkv // _HEADS_PER_DMA)),
            pltpu.SemaphoreType.DMA((len(_plan_wo(d, hd, ())[0]),)),
            pltpu.SemaphoreType.DMA((2,)),
        ],
        compiler_params=pltpu.CompilerParams(
            vmem_limit_bytes=32 * 1024 * 1024,
            disable_bounds_checks=True,
            disable_semaphore_checks=True,
        ),
        name="sliding_block_cached_sampling",
    )(
        x.reshape(rows, d),
        k_cache,
        v_cache,
        wq.reshape(w_shape),
        wo.T.reshape(w_shape),
    )
    return out.reshape(batch, sq, d)
```

```python
import functools
import math

import jax
import jax.numpy as jnp
from jax import lax
import jax.experimental.pallas as pl
import jax.experimental.pallas.tpu as pltpu

_HQ = 32
_TILE = 128
_RUN = 64
_HEADS_PER_DMA = 4
_SLOTS = 4
_WROWS = 64
_WCOLS = 512
_QUEUE = 26

_SMALL_KV = (5, 7)
_SMALL_LAST = 3
_WQ_AHEAD = 24
_WQ_LEAD = 15
_WO_SPLITS = ((9, 7), (6, 5, 5))

_NT = (((1,), (1,)), ((), ()))
_F32 = jnp.float32


def _ds(start, size):
    if not isinstance(start, int):
        start = pl.multiple_of(start, size)
    return pl.ds(start, size)


def _wait(filled, sem):
    pltpu.make_async_copy(filled, filled, sem).wait()


def _plan_wo(d, hd):
    blocks = d // _WROWS
    chunks = [(b, min(2, blocks - b)) for b in range(0, blocks, 2)][::-1]
    splits = [(16,)] * (len(chunks) - len(_WO_SPLITS)) + list(_WO_SPLITS)
    pieces = []
    for (b0, nb), split in zip(chunks, splits):
        c = 0
        for part in split:
            nc = hd * part // 16
            pieces.append((b0, nb, c, nc, nc // _WCOLS if nc == hd else 0))
            c += nc

    firsts = [0] * sum(_SMALL_KV) + [1] * (2 * _SMALL_LAST)
    firsts += [u + 2 for u, piece in enumerate(pieces) for _ in range(piece[4])]
    taken = [0] * len(pieces)
    small = []
    for first in firsts:
        for u in range(first, len(pieces)):
            b0, nb, c, nc, _ = pieces[u]
            per_row = nc // _WCOLS
            if nc == hd and taken[u] < nb * per_row:
                r, k = divmod(taken[u], per_row)
                small.append((u, b0, 1, 8 * r, 8, c + k * _WCOLS, _WCOLS))
                taken[u] += 1
                break
        else:
            small.append(None)

    bulk = []
    for u, (b0, nb, c, nc, _) in enumerate(pieces):
        full, part = divmod(taken[u], nc // _WCOLS)
        used = part * _WCOLS
        if nb == 1 or nc < hd // 2:
            for b in range(nb):
                r = 8 * full if b == 0 else 0
                if b == 0 and part:
                    bulk.append((u, b0, 1, r, 8, c + used, nc - used))
                    r += 8
                bulk.append((u, b0 + b, 1, r, _WROWS - r, c, nc))
            continue
        run = hd // 2 if nc % (hd // 2) == 0 else nc
        for r in range(0, _WROWS, 8):
            if r // 8 == full and part:
                bulk.append((u, b0, 1, r, 8, c + used, nc - used))
            if r // 8 < full + bool(part):
                bulk.append((u, b0 + 1, nb - 1, r, 8, c, nc))
            else:
                bulk += [(u, b0, nb, r, 8, k, run) for k in range(c, c + nc, run)]
    return pieces, bulk, small


def _kernel(
    x_hbm, k_hbm, v_hbm, wq_hbm, wot_hbm, o_hbm,
    x_s, wq_s, wot_s, kv_s, q_s, p_s, m_s, l_s, alpha_s, acc_s, att_s, part_s, out_s,
    x_sem, wq_sem, kv_sem, wo_sem, out_sem,
    *, window,
):
    batch, hkv, sk, dh = k_hbm.shape
    rows, d = x_hbm.shape
    hd = wq_hbm.shape[2]
    sq = rows // batch
    dtype = x_s.dtype
    tiles = window // _TILE
    steps = batch * tiles
    exp2_scale = dh ** -0.5 * math.log2(math.e)

    n_dmas = 2 * hkv // _HEADS_PER_DMA
    n_small = sum(_SMALL_KV)

    def locate(i):
        if isinstance(i, int):
            return i // tiles, i % tiles, i % _SLOTS
        b = lax.shift_right_logical(i, tiles.bit_length() - 1)
        return b, i & (tiles - 1), i & (_SLOTS - 1)

    def kv_copy(i, half, n, h0, nh, r0, nr):
        b, tile, slot = locate(i)
        group, a = divmod(n, 2)
        heads = pl.ds(group * _HEADS_PER_DMA + h0, nh)
        r = half * _RUN + r0
        src = (k_hbm, v_hbm)[a].at[
            b, heads, _ds(sk - window + tile * _TILE + r, nr), :
        ]
        dst = kv_s.at[slot, a, heads, pl.ds(r, nr), :]
        return pltpu.make_async_copy(src, dst, kv_sem.at[slot, half, n])

    def kv_bulk(i, half):
        for n in range(n_dmas):
            cut = len(range(n, n_small // 2, n_dmas))
            kv_copy(i, half, n, cut, _HEADS_PER_DMA - cut, 0, _RUN).start(priority=1)

    def kv_small(i, half, t):
        run, part = divmod(t, 2)
        kv_copy(
            i, half, run % n_dmas, run // n_dmas, 1, part * (_RUN // 2), _RUN // 2
        ).start(priority=0)

    def kv_wait(i, half, small=None):
        slot = locate(i)[2]
        first = n_dmas - 1 - _SMALL_KV[1]
        for n in range(n_dmas):
            group, a = divmod(n, 2)
            heads = pl.ds(group * _HEADS_PER_DMA, _HEADS_PER_DMA)
            _wait(
                kv_s.at[slot, a, heads, pl.ds(half * _RUN, _RUN), :],
                kv_sem.at[slot, half, n],
            )
            if small is not None and first <= n < n_dmas - 1:
                small(_SMALL_KV[0] + n - first)

    w_blocks = d // _WROWS
    wq_dmas = [
        (b0, b1, r, c)
        for r in range(0, _WROWS, 8)
        for c in range(0, hd, _WCOLS)
        for b0, b1 in ((0, w_blocks // 2), (w_blocks // 2, w_blocks))
    ]

    def wq_part(n, part):
        b0, b1, r, c = wq_dmas[n]
        if part == "small":
            b1 = b0 + 1
        elif part == "bulk" and n >= _WQ_LEAD:
            b0 += 1
        ix = pl.ds(b0, b1 - b0), pl.ds(r, 8), pl.ds(c, _WCOLS)
        return ix, wq_sem.at[n % _WQ_AHEAD]

    def wq_start(n, part):
        ix, sem = wq_part(n, part)
        pltpu.make_async_copy(wq_hbm.at[ix], wq_s.at[ix], sem).start(
            priority=int(part == "bulk")
        )

    pieces, wo_bulk, wo_small = _plan_wo(d, hd)
    wo_queued = []

    def wo_start(u, b0, nb, r, nr, c, nc, priority):
        ix = pl.ds(b0, nb), pl.ds(r, nr), pl.ds(c, nc)
        pltpu.make_async_copy(wot_hbm.at[ix], wot_s.at[ix], wo_sem.at[u]).start(
            priority=priority
        )

    def next_wo_bulk(count):
        for _ in range(min(count, len(wo_bulk))):
            wo_queued.append(wo_bulk.pop(0))
            wo_start(*wo_queued[-1], priority=1)

    def next_wo_small(_=None):
        entry = wo_small.pop(0)
        if entry is not None:
            wo_start(*entry, priority=0)

    def project_q(b, j0, nj):
        w = wq_s[:, :, _ds(j0 * 2 * dh, nj * 2 * dh)].reshape(d, nj * 2 * dh)
        q = jnp.dot(x_s[_ds(b * sq, sq), :], w, preferred_element_type=_F32)
        q = q.astype(dtype)
        for h in range(2 * nj):
            q_s[b & 1, j0 + h // 2, pl.ds((h % 2) * sq, sq), :] = (
                q[:, h * dh:(h + 1) * dh]
            )

    def reset_state():
        m_s[...] = jnp.full(m_s.shape, -jnp.inf, _F32)
        l_s[...] = jnp.zeros(l_s.shape, _F32)
        acc_s[...] = jnp.zeros(acc_s.shape, _F32)

    def all_matmuls(matmul, small, count):
        after = [int((t + 0.5) * hkv / count) for t in range(count)]
        results = []
        for j in range(hkv):
            results.append(matmul(j))
            if j in after:
                small(after.index(j))
        return results

    def scores_step(i, small, count=_SMALL_KV[0]):
        b, _, slot = locate(i)
        scores = all_matmuls(
            lambda j: lax.dot_general(
                q_s[b & 1, j], kv_s[slot, 0, j], _NT, preferred_element_type=_F32
            ),
            small,
            count,
        )
        for j, s in enumerate(scores):
            m_old = m_s[j]
            m_new = jnp.maximum(m_old, jnp.max(s, axis=1, keepdims=True))
            alpha = jnp.exp2((m_old - m_new) * exp2_scale)
            p = jnp.exp2((s - m_new) * exp2_scale)
            m_s[j] = m_new
            alpha_s[j] = alpha
            l_s[j] = alpha * l_s[j] + p
            p_s[j] = p.astype(dtype)

    def values_step(i, small, count=_SMALL_KV[0], next_q=True):
        b, tile, slot = locate(i)
        products = all_matmuls(
            lambda j: jnp.dot(
                p_s[j], kv_s[slot, 1, j], preferred_element_type=_F32
            ),
            small,
            count,
        )
        if next_q:
            project_q((b + 1) & (batch - 1), tile * (hkv // tiles), hkv // tiles)
        for j, pv in enumerate(products):
            acc_s[j] = alpha_s[j] * acc_s[j] + pv

    def finish_batch(b):
        for j in range(hkv):
            o = acc_s[j] / jnp.sum(l_s[j], axis=1, keepdims=True)
            o = o.astype(dtype)
            for h in range(2):
                att_s[j, b, :, pl.ds(h * dh, dh)] = o[h * sq:(h + 1) * sq]

    x_copy = pltpu.make_async_copy(x_hbm, x_s, x_sem)
    x_copy.start()
    for n in range(_WQ_AHEAD):
        wq_start(n, "bulk")
    reset_state()
    units = [(0, 0), (0, 1), (1, 0)]
    small = [(i, half, t) for i, half in units for t in range(n_small)]
    small = small[:len(small) - _SMALL_KV[1]]
    for n in range(len(wq_dmas)):
        ix, sem = wq_part(n, "all")
        _wait(wq_s.at[ix], sem)
        left = len(wq_dmas) - 1 - n
        if left >= _WQ_AHEAD:
            wq_start(n + _WQ_AHEAD, "bulk")
        elif units and left + n_dmas * (4 - len(units)) <= _QUEUE:
            kv_bulk(*units.pop(0))
        if left >= _WQ_LEAD:
            wq_start(n + _WQ_LEAD, "small")
        else:
            kv_small(*small.pop(0))
    assert not units
    x_copy.wait()
    groups = 4
    for n in range(groups):
        for _ in range(-(-len(small) // (groups - n))):
            kv_small(*small.pop(0))
        project_q(0, n * hkv // groups, hkv // groups)
        if n == groups // 2 - 1:
            kv_wait(0, 0)
            kv_bulk(1, 1)
    assert not small

    def step(i, _):
        kv_wait(i, 1, functools.partial(kv_small, i + 1, 0))
        kv_bulk(i + 2, 0)
        scores_step(i, functools.partial(kv_small, i + 1, 1))
        kv_wait(i + 1, 0, functools.partial(kv_small, i + 1, 1))
        kv_bulk(i + 2, 1)
        values_step(i, functools.partial(kv_small, i + 2, 0))
        b, tile, _ = locate(i)

        @pl.when(tile == tiles - 1)
        def _():
            finish_batch(b)
            reset_state()

    lax.fori_loop(0, steps - 2, step, None)

    i = steps - 2
    kv_wait(i, 1, functools.partial(kv_small, i + 1, 0))
    next_wo_bulk(_QUEUE - 2 * n_dmas)
    scores_step(i, functools.partial(kv_small, i + 1, 1))
    kv_wait(i + 1, 0, functools.partial(kv_small, i + 1, 1))
    next_wo_bulk(n_dmas)
    values_step(i, next_wo_small, next_q=False)
    i = steps - 1
    kv_wait(i, 1, next_wo_small)
    next_wo_bulk(n_dmas)
    scores_step(i, next_wo_small, _SMALL_LAST)
    values_step(i, next_wo_small, _SMALL_LAST, next_q=False)
    finish_batch(batch - 1)

    def out_copy(n, c, nc):
        cols = pl.ds(c, nc)
        return pltpu.make_async_copy(
            out_s.at[:, cols], o_hbm.at[:, cols], out_sem.at[n]
        )

    def project_out(b0, nb, c, nc, m, nm):
        att = jnp.concatenate(
            [
                att_s[j, pl.ds(m // sq, nm // sq)].reshape(nm, 2 * dh)
                for j in range(c // (2 * dh), (c + nc) // (2 * dh))
            ],
            axis=1,
        )
        w = wot_s[pl.ds(b0, nb), :, pl.ds(c, nc)].reshape(nb * _WROWS, nc)
        return lax.dot_general(att, w, _NT, preferred_element_type=_F32)

    last = pieces[-1][1] * _WROWS
    for u, (b0, nb, c, nc, count) in enumerate(pieces):
        assert all(entry[0] > u for entry in wo_bulk + wo_small if entry)
        _wait(wot_s.at[pl.ds(b0, nb), :, pl.ds(c, nc)], wo_sem.at[u])
        if u == len(pieces) - 1:
            out_copy(0, last, d - last).start()
        next_wo_bulk(_QUEUE - sum(entry[0] > u for entry in wo_queued))
        total = None
        for k in range(nc // _WCOLS):
            if k < count:
                next_wo_small()
            part = project_out(b0, nb, c + k * _WCOLS, _WCOLS, 0, rows)
            total = part if total is None else total + part
        rest = nc % _WCOLS
        if rest:
            total += jnp.concatenate(
                [
                    project_out(b0, nb, c + nc - rest, rest, m, rows // 2)
                    for m in (0, rows // 2)
                ],
                axis=0,
            )
        if c > 0:
            total += part_s[...]
        if c + nc < hd:
            part_s[...] = total
        else:
            out_s[:, pl.ds(b0 * _WROWS, nb * _WROWS)] = total.astype(out_s.dtype)
    assert not wo_bulk and not wo_small
    out_copy(1, 0, last).start()
    out_copy(0, last, d - last).wait()
    out_copy(1, 0, last).wait()


@jax.jit
def pallas_standalone__sliding_block_cached__sampling_kernel(
    x: jax.Array,
    k_cache: jax.Array,
    v_cache: jax.Array,
    wq: jax.Array,
    wo: jax.Array,
):
    batch, sq, d = x.shape
    _, hkv, sk, dh = k_cache.shape
    window = min(4096, max(256, sk // 4))
    tiles = window // _TILE
    assert _HQ == 2 * hkv and d % _WROWS == 0
    assert window % _TILE == 0 and sk % _TILE == 0 and hkv % tiles == 0
    assert tiles & (tiles - 1) == 0 and batch & (batch - 1) == 0 and batch > 1
    rows, hd, dtype = batch * sq, _HQ * dh, x.dtype
    w_shape = (d // _WROWS, _WROWS, hd)

    hbm = pl.BlockSpec(memory_space=pl.ANY)
    state = pltpu.VMEM((hkv, 2 * sq, dh), _F32)
    out = pl.pallas_call(
        functools.partial(_kernel, window=window),
        out_shape=jax.ShapeDtypeStruct((rows, d), dtype),
        in_specs=[hbm] * 5,
        out_specs=hbm,
        scratch_shapes=[
            pltpu.VMEM((rows, d), dtype),
            pltpu.VMEM(w_shape, dtype),
            pltpu.VMEM(w_shape, dtype),
            pltpu.VMEM((_SLOTS, 2, hkv, _TILE, dh), dtype),
            pltpu.VMEM((2, hkv, 2 * sq, dh), dtype),
            pltpu.VMEM((hkv, 2 * sq, dh), dtype),
            state,
            state,
            state,
            state,
            pltpu.VMEM((hkv, batch, sq, 2 * dh), dtype),
            pltpu.VMEM((rows, 2 * _WROWS), _F32),
            pltpu.VMEM((rows, d), dtype),
            pltpu.SemaphoreType.DMA,
            pltpu.SemaphoreType.DMA((_WQ_AHEAD,)),
            pltpu.SemaphoreType.DMA((_SLOTS, 2, 2 * hkv // _HEADS_PER_DMA)),
            pltpu.SemaphoreType.DMA((len(_plan_wo(d, hd)[0]),)),
            pltpu.SemaphoreType.DMA((2,)),
        ],
        compiler_params=pltpu.CompilerParams(
            vmem_limit_bytes=32 * 1024 * 1024,
            disable_semaphore_checks=True,
        ),
        name="sliding_block_cached_sampling",
    )(
        x.reshape(rows, d),
        k_cache,
        v_cache,
        wq.reshape(w_shape),
        wo.T.reshape(w_shape),
    )
    return out.reshape(batch, sq, d)
```
